```python
import jax
import jax.numpy as jnp

def _softmax(x, axis=-1):
    return jax.nn.softmax(x, axis=axis)

def _gelu(x):
    return jax.nn.gelu(x, approximate=True)

def _silu(x):
    return jax.nn.silu(x)

def _sigmoid(x):
    return jax.nn.sigmoid(x)

def _layernorm(x, axis=-1, eps=1e-05):
    m = jnp.mean(x, axis=axis, keepdims=True)
    v = jnp.var(x, axis=axis, keepdims=True)
    return (x - m) / jnp.sqrt(v + eps)

def _scatter_add(tgt, idx, src, axis=0):
    return tgt.at[idx].add(src)

def _segment_sum(src, seg, n):
    return jax.ops.segment_sum(src, seg, n)

class _Rng:

    def __init__(self, key):
        self._k = key

    def _next(self):
        self._k, sub = jax.random.split(self._k)
        return sub

    def normal(self, shape):
        return jax.random.normal(self._next(), shape, dtype=jnp.bfloat16)

    def randint(self, lo, hi, shape):
        return jax.random.randint(self._next(), shape, lo, hi, dtype=jnp.int32)

    def uniform(self, shape, lo=0.0, hi=1.0):
        return jax.random.uniform(self._next(), shape, jnp.bfloat16, lo, hi)

    def permutation(self, n):
        return jax.random.permutation(self._next(), n)
kernel_name = 'concat_heads__compressed_kv_cla__memory_aug_recurrent_mem_tr__prompt'

def setup_inputs():
    _rng = _Rng(jax.random.key(int.from_bytes(__import__("os").urandom(4), "little")))
    _w = lambda a: (lambda t: t.astype(jnp.bfloat16) if jnp.issubdtype(t.dtype, jnp.floating) else t)(jnp.asarray(a))

    def _A_setup():
        B, H, Sq, Sk, D, M = (1, 32, 2048, 2048, 128, 576)
        Dc = 4 * D
        return {'x': _w((lambda *s: _rng.normal(s) * 0.05)(B, Sq, M)), 'c_kv': _w((lambda *s: _rng.normal(s) * 0.05)(B, Sk, Dc)), 'w_q': _w((lambda *s: _rng.normal(s) * 0.05)(M, H, D) * M ** (-0.5)), 'w_uk': _w((lambda *s: _rng.normal(s) * 0.05)(Dc, H, D) * Dc ** (-0.5)), 'w_uv': _w((lambda *s: _rng.normal(s) * 0.05)(Dc, H, D) * Dc ** (-0.5)), 'w_o': _w((lambda *s: _rng.normal(s) * 0.05)(H, D, M) * (H * D) ** (-0.5))}
    _A_in = _A_setup()

    def _B_setup():
        B, S, Dm = (1, 2048, 576)
        H, Dh = (32, 128)
        M, seg = (8, 32)
        seg = min(seg, S)
        S = S // seg * seg
        return {'x': _w((lambda *s: _rng.normal(s) * 0.05)(B, S, Dm)), 'mem0': _w((lambda *s: _rng.normal(s) * 0.05)(B, M, Dm)), 'Wq': _w((lambda *s: _rng.normal(s) * 0.05)(Dm, H, Dh) * Dm ** (-0.5)), 'Wk': _w((lambda *s: _rng.normal(s) * 0.05)(Dm, H, Dh) * Dm ** (-0.5)), 'Wv': _w((lambda *s: _rng.normal(s) * 0.05)(Dm, H, Dh) * Dm ** (-0.5)), 'Wo': _w((lambda *s: _rng.normal(s) * 0.05)(H, Dh, Dm) * (H * Dh) ** (-0.5)), 'seg_len': seg}
    _B_in = _B_setup()
    return {'A_x': _A_in['x'], 'A_c_kv': _A_in['c_kv'], 'A_w_q': _A_in['w_q'], 'A_w_uk': _A_in['w_uk'], 'A_w_uv': _A_in['w_uv'], 'A_w_o': _A_in['w_o'], 'B_x': _B_in['x'], 'B_mem0': _B_in['mem0'], 'B_Wq': _B_in['Wq'], 'B_Wk': _B_in['Wk'], 'B_Wv': _B_in['Wv'], 'B_Wo': _B_in['Wo'], 'B_seg_len': _B_in['seg_len']}

def reference(A_x, A_c_kv, A_w_q, A_w_uk, A_w_uv, A_w_o, B_x, B_mem0, B_Wq, B_Wk, B_Wv, B_Wo, B_seg_len):

    def _A_ref(x, c_kv, w_q, w_uk, w_uv, w_o):
        B, Sq, M = (x.shape[0], x.shape[1], x.shape[2])
        Sk = c_kv.shape[1]
        H, D = (w_q.shape[1], w_q.shape[2])
        q = jnp.einsum('bqm,mhd->bhqd', x, w_q)
        k = jnp.einsum('bkc,chd->bhkd', c_kv, w_uk)
        v = jnp.einsum('bkc,chd->bhkd', c_kv, w_uv)
        scores = jnp.einsum('bhqd,bhkd->bhqk', q, k) * D ** (-0.5)
        off = Sk - Sq
        qi = jnp.arange(Sq)[:, None]
        kj = jnp.arange(Sk)[None, :]
        cmask = kj <= qi + off
        scores = jnp.where(cmask[None, None], scores, -1000000000.0)
        p = _softmax(scores, axis=-1)
        ctx = jnp.einsum('bhqk,bhkd->bhqd', p, v)
        return jnp.einsum('bhqd,hdm->bqm', ctx, w_o)

    def _B_ref(x, mem0, Wq, Wk, Wv, Wo, seg_len):
        B, S, Dm = x.shape
        H, Dh = (Wq.shape[1], Wq.shape[2])
        M = mem0.shape[1]
        scale = Dh ** (-0.5)
        n_seg = S // seg_len
        L = M + seg_len
        idx = jnp.arange(L)
        mask = (idx[:, None] < M) | (idx[:, None] >= idx[None, :])
        mem = mem0
        outs = []
        for s in range(n_seg):
            xs = x[:, s * seg_len:(s + 1) * seg_len, :].copy()
            h = jnp.concatenate([mem, xs], axis=1)
            q = jnp.einsum('btd,dhe->bhte', h, Wq)
            k = jnp.einsum('btd,dhe->bhte', h, Wk)
            v = jnp.einsum('btd,dhe->bhte', h, Wv)
            scores = jnp.einsum('bhqe,bhke->bhqk', q, k) * scale
            scores = jnp.where(mask[None, None], scores, -1000000000.0)
            p = _softmax(scores, axis=-1)
            o = jnp.einsum('bhqk,bhke->bhqe', p, v)
            o = jnp.einsum('bhte,hed->btd', o, Wo)
            mem = o[:, :M, :].copy()
            outs.append(o[:, M:, :])
        return jnp.concatenate(outs, axis=1)
    a = _A_ref(A_x, A_c_kv, A_w_q, A_w_uk, A_w_uv, A_w_o)
    b = _B_ref(B_x, B_mem0, B_Wq, B_Wk, B_Wv, B_Wo, B_seg_len)
    return jnp.concatenate([a, b], axis=-1)
```

```python
import functools
import math

import jax
import jax.numpy as jnp
from jax import lax
import jax.experimental.pallas as pl
import jax.experimental.pallas.tpu as pltpu

S = 2048
DM = 576
DC = 512
H = 32
DH = 128
HD = H * DH
MEM = 8
SEG = 32
NSEG = S // SEG
NEG = -1e9
LOG2E = math.log2(math.e)
QSCALE = DH ** -0.5 * LOG2E

BF = jnp.bfloat16
F32 = jnp.float32
NT = (((1,), (1,)), ((), ()))


def _dot(a, b):
    return jnp.dot(a, b, preferred_element_type=F32)


def _dot_nt(a, b):
    return lax.dot_general(a, b, NT, preferred_element_type=F32)


def _kernel(ax_h, ckv_h, awq_h, awk_h, awv_h, awo_h, bx_h, mem0_ref, bwq_h, bwk_h, bwv_h, bwo_h,
            o_ref,
            ax, ckv, bx, raw0, raw1, raw2, awo, bwo, wq2, wk2, wv2, kx, vx, kmem, vmem, ctxa, sems):
    def cp(src, dst, i):
        return pltpu.make_async_copy(src, dst, sems.at[i])

    c_bx = cp(bx_h, bx, 0)
    c_bwk = cp(bwk_h, raw0, 1)
    c_bwv = cp(bwv_h, raw1, 2)
    c_bwq = cp(bwq_h, raw2, 3)
    c_bwo = cp(bwo_h, bwo, 4)
    c_ax = cp(ax_h, ax, 5)
    c_ckv = cp(ckv_h, ckv, 6)
    c_awo = cp(awo_h, awo, 7)
    c_awq = cp(awq_h, raw0, 8)
    c_awk = cp(awk_h, raw1.at[pl.ds(0, DC)], 9)
    c_awv = cp(awv_h, raw2.at[pl.ds(0, DC)], 10)
    for c in (c_bx, c_bwk, c_bwv, c_bwq, c_bwo, c_ax, c_ckv, c_awo):
        c.start()

    RB = 512
    c_bx.wait()
    for c_in, c_next, raw, w2, dst in ((c_bwk, c_awq, raw0, wk2, kx), (c_bwv, c_awk, raw1, wv2, vx)):
        c_in.wait()
        for g in range(2):
            w2[:, g * 2048:(g + 1) * 2048] = raw[:, g * 16:(g + 1) * 16, :].reshape(DM, 2048)
        c_next.start()

        def proj(r, carry, w2=w2, dst=dst):
            rows = pl.ds(pl.multiple_of(r * RB, RB), RB)
            xr = bx[rows, :]
            for g in range(4):
                cols = slice(g * 1024, (g + 1) * 1024)
                dst[rows, cols] = _dot(xr, w2[:, cols]).astype(BF)
            return carry
        lax.fori_loop(0, S // RB, proj, 0)
    c_bwq.wait()
    for g in range(2):
        wq2[:, g * 2048:(g + 1) * 2048] = raw2[:, g * 16:(g + 1) * 16, :].reshape(DM, 2048)
    c_awv.start()
    c_bwo.wait()

    def mem_step(mem, s):
        q = _dot(mem, wq2[...]) * QSCALE
        k = _dot(mem, wk2[...])
        v = _dot(mem, wv2[...])
        rows = pl.ds(pl.multiple_of(s * SEG, SEG), SEG)
        ctx = []
        for h in range(H):
            cs = slice(h * DH, (h + 1) * DH)
            qh = q[:, cs].astype(BF)
            s_m = _dot_nt(qh, k[:, cs].astype(BF))
            s_x = _dot_nt(qh, kx[rows, cs])
            m = jnp.maximum(jnp.max(s_m, axis=1, keepdims=True), jnp.max(s_x, axis=1, keepdims=True))
            p_m = jnp.exp2(s_m - m)
            p_x = jnp.exp2(s_x - m)
            l = jnp.sum(p_m, axis=1, keepdims=True) + jnp.sum(p_x, axis=1, keepdims=True)
            o = _dot(p_m.astype(BF), v[:, cs].astype(BF)) + _dot(p_x.astype(BF), vx[rows, cs])
            ctx.append(o / l)
        ctx = jnp.concatenate(ctx, axis=1).astype(BF)
        return _dot(ctx, bwo[...]).astype(BF), k, v

    def rec(p, mem):
        mem1, k0, v0 = mem_step(mem, 2 * p)
        mem2, k1, v1 = mem_step(mem1, 2 * p + 1)
        prow = pl.ds(pl.multiple_of(p * 16, 16), 16)
        kmem[prow, :] = jnp.concatenate([k0, k1], axis=0).astype(BF)
        vmem[prow, :] = jnp.concatenate([v0, v1], axis=0).astype(BF)
        return mem2
    lax.fori_loop(0, NSEG // 2, rec, mem0_ref[...])

    c_ax.wait(); c_ckv.wait(); c_awq.wait(); c_awk.wait(); c_awv.wait()
    BQ = 256
    tri = (lax.broadcasted_iota(jnp.int32, (BQ, BQ), 1) <= lax.broadcasted_iota(jnp.int32, (BQ, BQ), 0))

    def head_pair(raw, rows, i):
        u = raw.bitcast(jnp.uint32)[0:rows, pl.ds(i, 1), :].reshape(rows, DH)
        lo = pltpu.bitcast(u << 16, F32).astype(BF)
        hi = pltpu.bitcast(u & jnp.uint32(0xFFFF0000), F32).astype(BF)
        return lo, hi

    def a_pair(i2, carry):
        wq = head_pair(raw0, DM, i2)
        wk = head_pair(raw1, DC, i2)
        wv = head_pair(raw2, DC, i2)
        for e in range(2):
            cols = pl.ds(pl.multiple_of(i2 * 2 * DH + e * DH, DH), DH)
            q = (_dot(ax[...], wq[e]) * QSCALE).astype(BF)
            k = _dot(ckv[...], wk[e]).astype(BF)
            v = _dot(ckv[...], wv[e]).astype(BF)
            for i in range(S // BQ):
                r0 = i * BQ
                qi = q[r0:r0 + BQ]
                sd = jnp.where(tri, _dot_nt(qi, k[r0:r0 + BQ]), NEG)
                m = jnp.max(sd, axis=1, keepdims=True)
                if i > 0:
                    so = _dot_nt(qi, k[0:r0])
                    m = jnp.maximum(m, jnp.max(so, axis=1, keepdims=True))
                pd = jnp.exp2(sd - m)
                l = jnp.sum(pd, axis=1, keepdims=True)
                o = _dot(pd.astype(BF), v[r0:r0 + BQ])
                if i > 0:
                    po = jnp.exp2(so - m)
                    l = l + jnp.sum(po, axis=1, keepdims=True)
                    o = o + _dot(po.astype(BF), v[0:r0])
                ctxa[r0:r0 + BQ, cols] = (o / l).astype(BF)
        return carry
    lax.fori_loop(0, H // 2, a_pair, 0)

    c_awo.wait()

    def a_out(r, carry):
        rows = pl.ds(pl.multiple_of(r * RB, RB), RB)
        o_ref[rows, 0:DM] = _dot(ctxa[rows, :], awo[...]).astype(BF)
        return carry
    lax.fori_loop(0, S // RB, a_out, 0)

    ri = lax.broadcasted_iota(jnp.int32, (2 * SEG, 2 * (MEM + SEG)), 0)
    ci = lax.broadcasted_iota(jnp.int32, (2 * SEG, 2 * (MEM + SEG)), 1)
    rseg = ri // SEG
    vis = jnp.where(ci < 2 * MEM, (ci // MEM == rseg).astype(jnp.int32),
                    (((ci - 2 * MEM) // SEG == rseg) & (ci - 2 * MEM <= ri)).astype(jnp.int32)) > 0

    def b_head(h, carry):
        cols = pl.ds(pl.multiple_of(h * DH, DH), DH)
        q = (_dot(bx[...], wq2[:, cols]) * QSCALE).astype(BF)
        for p in range(NSEG // 2):
            xr = slice(p * 64, (p + 1) * 64)
            mr = slice(p * 16, (p + 1) * 16)
            kk = jnp.concatenate([kmem[mr, cols], kx[xr, cols]], axis=0)
            vv = jnp.concatenate([vmem[mr, cols], vx[xr, cols]], axis=0)
            s = jnp.where(vis, _dot_nt(q[xr], kk), NEG)
            m = jnp.max(s, axis=1, keepdims=True)
            pr = jnp.exp2(s - m)
            l = jnp.sum(pr, axis=1, keepdims=True)
            o = _dot(pr.astype(BF), vv) / l
            ctxa[xr, cols] = o.astype(BF)
        return carry
    lax.fori_loop(0, H, b_head, 0)

    def b_out(r, carry):
        rows = pl.ds(pl.multiple_of(r * RB, RB), RB)
        o_ref[rows, DM:2 * DM] = _dot(ctxa[rows, :], bwo[...]).astype(BF)
        return carry
    lax.fori_loop(0, S // RB, b_out, 0)


@jax.jit
def _run(A_x, A_c_kv, A_w_q, A_w_uk, A_w_uv, A_w_o, B_x, B_mem0, B_Wq, B_Wk, B_Wv, B_Wo):
    any_spec = pl.BlockSpec(memory_space=pl.ANY)
    vm = pltpu.VMEM
    out = pl.pallas_call(
        _kernel,
        out_shape=jax.ShapeDtypeStruct((S, 2 * DM), BF),
        in_specs=[any_spec] * 7 + [pl.BlockSpec(memory_space=pltpu.VMEM)] + [any_spec] * 4,
        out_specs=pl.BlockSpec(memory_space=pltpu.VMEM),
        scratch_shapes=[
            vm((S, DM), BF), vm((S, DC), BF), vm((S, DM), BF),
            vm((DM, H, DH), BF), vm((DM, H, DH), BF), vm((DM, H, DH), BF),
            vm((HD, DM), BF), vm((HD, DM), BF),
            vm((DM, HD), BF), vm((DM, HD), BF), vm((DM, HD), BF),
            vm((S, HD), BF), vm((S, HD), BF),
            vm((NSEG * MEM, HD), BF), vm((NSEG * MEM, HD), BF),
            vm((S, HD), BF),
            pltpu.SemaphoreType.DMA((11,)),
        ],
        compiler_params=pltpu.CompilerParams(vmem_limit_bytes=126 * 2 ** 20),
    )(A_x.reshape(S, DM), A_c_kv.reshape(S, DC), A_w_q, A_w_uk, A_w_uv, A_w_o.reshape(HD, DM),
      B_x.reshape(S, DM), B_mem0.reshape(MEM, DM), B_Wq, B_Wk, B_Wv, B_Wo.reshape(HD, DM))
    return out.reshape(1, S, 2 * DM)


def pallas_concat_heads__compressed_kv_cla__memory_aug_recurrent_mem_tr__prompt_kernel(
        A_x, A_c_kv, A_w_q, A_w_uk, A_w_uv, A_w_o, B_x, B_mem0, B_Wq, B_Wk, B_Wv, B_Wo, B_seg_len=SEG):
    del B_seg_len
    return _run(A_x, A_c_kv, A_w_q, A_w_uk, A_w_uv, A_w_o, B_x, B_mem0, B_Wq, B_Wk, B_Wv, B_Wo)
```

```python
import functools
import math

import jax
import jax.numpy as jnp
from jax import lax
import jax.experimental.pallas as pl
import jax.experimental.pallas.tpu as pltpu

S = 2048
DM = 576
DC = 512
H = 32
DH = 128
HD = H * DH
MEM = 8
SEG = 32
NSEG = S // SEG
NEG = -1e9
LOG2E = math.log2(math.e)
QSCALE = DH ** -0.5 * LOG2E

BF = jnp.bfloat16
F32 = jnp.float32
NT = (((1,), (1,)), ((), ()))


def _dot(a, b):
    return jnp.dot(a, b, preferred_element_type=F32)


def _dot_nt(a, b):
    return lax.dot_general(a, b, NT, preferred_element_type=F32)


def _kernel(ax_h, ckv_h, awq_h, awk_h, awv_h, awo_h, bx_h, mem0_ref, bwq_h, bwk_h, bwv_h, bwo_h,
            o_ref,
            ax, ckv, bx, raw0, raw1, raw2, awo, bwo, wq2, wk2, wv2, kx, vx, kmem, vmem, ctxa, sems, wsems):
    def cp(src, dst, i):
        return pltpu.make_async_copy(src, dst, sems.at[i])

    c_bx = cp(bx_h, ctxa.at[0:DM, 0:S], 0)
    c_bwk = cp(bwk_h, raw0, 1)
    c_bwv = cp(bwv_h, raw1, 2)
    c_bwq = cp(bwq_h, raw2, 3)
    c_bwo = [pltpu.make_async_copy(bwo_h.at[h], ctxa.at[1024:1024 + DM, h * DH:(h + 1) * DH], wsems.at[h]) for h in range(H)]
    c_ax = cp(ax_h, ctxa.at[0:DM, S:2 * S], 5)
    c_ckv = cp(ckv_h, ckv, 6)
    c_awo = [pltpu.make_async_copy(awo_h.at[h], awo.at[:, h * DH:(h + 1) * DH], wsems.at[H + h])
             for h in range(H)]
    c_awq = cp(awq_h, raw0, 8)
    c_awk = cp(awk_h, raw1.at[pl.ds(0, DC)], 9)
    c_awv = cp(awv_h, raw2.at[pl.ds(0, DC)], 10)
    for c in (c_bx, c_bwk, c_bwv, c_bwq, *c_bwo, c_ax, c_ckv):
        c.start()

    RB = 512
    c_bx.wait()

    def untranspose_x(dst, c0):
        for r in range(S // 128):
            xt = ctxa[0:DM, c0 + r * 128:c0 + (r + 1) * 128].astype(F32)
            dst[r * 128:(r + 1) * 128, :] = xt.T.astype(BF)
    untranspose_x(bx, 0)
    for c_in, c_next, raw, w2, dst in ((c_bwk, c_awq, raw0, wk2, kx), (c_bwv, c_awk, raw1, wv2, vx)):
        c_in.wait()
        for g in range(2):
            w2[:, g * 2048:(g + 1) * 2048] = raw[:, g * 16:(g + 1) * 16, :].reshape(DM, 2048)
        c_next.start()

        def proj(r, carry, w2=w2, dst=dst):
            rows = pl.ds(pl.multiple_of(r * RB, RB), RB)
            xr = bx[rows, :]
            for g in range(4):
                cols = slice(g * 1024, (g + 1) * 1024)
                dst[rows, cols] = _dot(xr, w2[:, cols]).astype(BF)
            return carry
        lax.fori_loop(0, S // RB, proj, 0)
    c_bwq.wait()
    for g in range(2):
        wq2[:, g * 2048:(g + 1) * 2048] = raw2[:, g * 16:(g + 1) * 16, :].reshape(DM, 2048)
    c_awv.start()
    for c in c_bwo:
        c.wait()
    for h in range(H):
        bwo[h * DH:(h + 1) * DH, :] = ctxa[1024:1024 + DM, h * DH:(h + 1) * DH].astype(F32).T.astype(BF)
    for c in c_awo:
        c.start()

    def mem_step(mem, s):
        q = _dot(mem, wq2[...]) * QSCALE
        k = _dot(mem, wk2[...])
        v = _dot(mem, wv2[...])
        rows = pl.ds(pl.multiple_of(s * SEG, SEG), SEG)
        ctx = []
        for h in range(H):
            cs = slice(h * DH, (h + 1) * DH)
            qh = q[:, cs].astype(BF)
            s_m = _dot_nt(qh, k[:, cs].astype(BF))
            s_x = _dot_nt(qh, kx[rows, cs])
            m = jnp.maximum(jnp.max(s_m, axis=1, keepdims=True), jnp.max(s_x, axis=1, keepdims=True))
            p_m = jnp.exp2(s_m - m)
            p_x = jnp.exp2(s_x - m)
            l = jnp.sum(p_m, axis=1, keepdims=True) + jnp.sum(p_x, axis=1, keepdims=True)
            o = _dot(p_m.astype(BF), v[:, cs].astype(BF)) + _dot(p_x.astype(BF), vx[rows, cs])
            ctx.append(o / l)
        ctx = jnp.concatenate(ctx, axis=1).astype(BF)
        return _dot(ctx, bwo[...]).astype(BF), k, v

    def rec(p, mem):
        mem1, k0, v0 = mem_step(mem, 2 * p)
        mem2, k1, v1 = mem_step(mem1, 2 * p + 1)
        prow = pl.ds(pl.multiple_of(p * 16, 16), 16)
        kmem[prow, :] = jnp.concatenate([k0, k1], axis=0).astype(BF)
        vmem[prow, :] = jnp.concatenate([v0, v1], axis=0).astype(BF)
        return mem2
    lax.fori_loop(0, NSEG // 2, rec, mem0_ref[...])

    c_ax.wait(); c_ckv.wait(); c_awq.wait(); c_awk.wait(); c_awv.wait()
    untranspose_x(ax, S)
    BQ = 256
    tri = (lax.broadcasted_iota(jnp.int32, (BQ, BQ), 1) <= lax.broadcasted_iota(jnp.int32, (BQ, BQ), 0))

    def head_pair(raw, rows, i):
        u = raw.bitcast(jnp.uint32)[0:rows, pl.ds(i, 1), :].reshape(rows, DH)
        lo = pltpu.bitcast(u << 16, F32).astype(BF)
        hi = pltpu.bitcast(u & jnp.uint32(0xFFFF0000), F32).astype(BF)
        return lo, hi

    def a_pair(i2, carry):
        wq = head_pair(raw0, DM, i2)
        wk = head_pair(raw1, DC, i2)
        wv = head_pair(raw2, DC, i2)
        for e in range(2):
            cols = pl.ds(pl.multiple_of(i2 * 2 * DH + e * DH, DH), DH)
            q = (_dot(ax[...], wq[e]) * QSCALE).astype(BF)
            k = _dot(ckv[...], wk[e]).astype(BF)
            v = _dot(ckv[...], wv[e]).astype(BF)
            for i in range(S // BQ):
                r0 = i * BQ
                qi = q[r0:r0 + BQ]
                sd = jnp.where(tri, _dot_nt(qi, k[r0:r0 + BQ]), NEG)
                m = jnp.max(sd, axis=1, keepdims=True)
                if i > 0:
                    so = _dot_nt(qi, k[0:r0])
                    m = jnp.maximum(m, jnp.max(so, axis=1, keepdims=True))
                pd = jnp.exp2(sd - m)
                l = jnp.sum(pd, axis=1, keepdims=True)
                o = _dot(pd.astype(BF), v[r0:r0 + BQ])
                if i > 0:
                    po = jnp.exp2(so - m)
                    l = l + jnp.sum(po, axis=1, keepdims=True)
                    o = o + _dot(po.astype(BF), v[0:r0])
                ctxa[r0:r0 + BQ, cols] = (o / l).astype(BF)
        return carry
    lax.fori_loop(0, H // 2, a_pair, 0)

    for c in c_awo:
        c.wait()

    def a_out(r, carry):
        rows = pl.ds(pl.multiple_of(r * RB, RB), RB)
        o_ref[rows, 0:DM] = _dot_nt(ctxa[rows, :], awo[...]).astype(BF)
        return carry
    lax.fori_loop(0, S // RB, a_out, 0)

    ri = lax.broadcasted_iota(jnp.int32, (2 * SEG, 2 * (MEM + SEG)), 0)
    ci = lax.broadcasted_iota(jnp.int32, (2 * SEG, 2 * (MEM + SEG)), 1)
    rseg = ri // SEG
    vis = jnp.where(ci < 2 * MEM, (ci // MEM == rseg).astype(jnp.int32),
                    (((ci - 2 * MEM) // SEG == rseg) & (ci - 2 * MEM <= ri)).astype(jnp.int32)) > 0

    def b_head(h, carry):
        cols = pl.ds(pl.multiple_of(h * DH, DH), DH)
        q = (_dot(bx[...], wq2[:, cols]) * QSCALE).astype(BF)
        for p in range(NSEG // 2):
            xr = slice(p * 64, (p + 1) * 64)
            mr = slice(p * 16, (p + 1) * 16)
            kk = jnp.concatenate([kmem[mr, cols], kx[xr, cols]], axis=0)
            vv = jnp.concatenate([vmem[mr, cols], vx[xr, cols]], axis=0)
            s = jnp.where(vis, _dot_nt(q[xr], kk), NEG)
            m = jnp.max(s, axis=1, keepdims=True)
            pr = jnp.exp2(s - m)
            l = jnp.sum(pr, axis=1, keepdims=True)
            o = _dot(pr.astype(BF), vv) / l
            ctxa[xr, cols] = o.astype(BF)
        return carry
    lax.fori_loop(0, H, b_head, 0)

    def b_out(r, carry):
        rows = pl.ds(pl.multiple_of(r * RB, RB), RB)
        o_ref[rows, DM:2 * DM] = _dot(ctxa[rows, :], bwo[...]).astype(BF)
        return carry
    lax.fori_loop(0, S // RB, b_out, 0)


@jax.jit
def _run(A_x, A_c_kv, A_w_q, A_w_uk, A_w_uv, A_w_o, B_x, B_mem0, B_Wq, B_Wk, B_Wv, B_Wo):
    any_spec = pl.BlockSpec(memory_space=pl.ANY)
    vm = pltpu.VMEM
    out = pl.pallas_call(
        _kernel,
        out_shape=jax.ShapeDtypeStruct((S, 2 * DM), BF),
        in_specs=[any_spec] * 7 + [pl.BlockSpec(memory_space=pltpu.VMEM)] + [any_spec] * 4,
        out_specs=pl.BlockSpec(memory_space=pltpu.VMEM),
        scratch_shapes=[
            vm((S, DM), BF), vm((S, DC), BF), vm((S, DM), BF),
            vm((DM, H, DH), BF), vm((DM, H, DH), BF), vm((DM, H, DH), BF),
            vm((DM, HD), BF), vm((HD, DM), BF),
            vm((DM, HD), BF), vm((DM, HD), BF), vm((DM, HD), BF),
            vm((S, HD), BF), vm((S, HD), BF),
            vm((NSEG * MEM, HD), BF), vm((NSEG * MEM, HD), BF),
            vm((S, HD), BF),
            pltpu.SemaphoreType.DMA((11,)),
            pltpu.SemaphoreType.DMA((2 * H,)),
        ],
        compiler_params=pltpu.CompilerParams(vmem_limit_bytes=126 * 2 ** 20),
    )(A_x.reshape(S, DM).T, A_c_kv.reshape(S, DC), A_w_q, A_w_uk, A_w_uv, jnp.transpose(A_w_o, (0, 2, 1)),
      B_x.reshape(S, DM).T, B_mem0.reshape(MEM, DM), B_Wq, B_Wk, B_Wv, jnp.transpose(B_Wo, (0, 2, 1)))
    return out.reshape(1, S, 2 * DM)


def pallas_concat_heads__compressed_kv_cla__memory_aug_recurrent_mem_tr__prompt_kernel(
        A_x, A_c_kv, A_w_q, A_w_uk, A_w_uv, A_w_o, B_x, B_mem0, B_Wq, B_Wk, B_Wv, B_Wo, B_seg_len=SEG):
    del B_seg_len
    return _run(A_x, A_c_kv, A_w_q, A_w_uk, A_w_uv, A_w_o, B_x, B_mem0, B_Wq, B_Wk, B_Wv, B_Wo)
```

```python
import functools
import math

import jax
import jax.numpy as jnp
from jax import lax
import jax.experimental.pallas as pl
import jax.experimental.pallas.tpu as pltpu

S = 2048
DM = 576
DC = 512
H = 32
DH = 128
HD = H * DH
MEM = 8
SEG = 32
NSEG = S // SEG
NEG = -1e9
LOG2E = math.log2(math.e)
QSCALE = DH ** -0.5 * LOG2E

BF = jnp.bfloat16
F32 = jnp.float32
NT = (((1,), (1,)), ((), ()))


def _dot(a, b):
    return jnp.dot(a, b, preferred_element_type=F32)


def _dot_nt(a, b):
    return lax.dot_general(a, b, NT, preferred_element_type=F32)


def _recip(l):
    r = pl.reciprocal(l, approx=True)
    return r * (2.0 - l * r)


def _w(ref, rows=slice(None), cols=slice(None)):
    return pltpu.bitcast(ref[rows, cols], BF)


def _kernel(ax_h, ckv_h, awq_h, awk_h, awv_h, awo_h, bx_h, mem0_ref, bwq_h, bwk_h, bwv_h, bwo_h,
            o_ref,
            ax, ckv, bx, raw0, raw1, raw2, awo, bwo, wq2, wk2, wv2, kx, vx, kmem, vmem, ctxa, sems, wsems):
    def cp(src, dst, i):
        return pltpu.make_async_copy(src, dst, sems.at[i])

    c_bx = cp(bx_h, ctxa.at[0:DM, 0:S], 0)
    c_bwk = cp(bwk_h, raw0, 1)
    c_bwv = cp(bwv_h, raw1, 2)
    c_bwq = cp(bwq_h, raw2, 3)
    c_bwo = [pltpu.make_async_copy(bwo_h.at[h], ctxa.at[1024:1024 + DM, h * DH:(h + 1) * DH], wsems.at[h])
             for h in range(H)]
    c_ax = cp(ax_h, ctxa.at[0:DM, S:2 * S], 5)
    c_ckv = cp(ckv_h, ckv, 6)
    c_awo = [pltpu.make_async_copy(awo_h.at[h], awo.at[:, h * DH:(h + 1) * DH], wsems.at[H + h])
             for h in range(H)]
    c_awq = cp(awq_h, raw0, 8)
    c_awk = cp(awk_h, raw1.at[pl.ds(0, DC)], 9)
    c_awv = cp(awv_h, raw2.at[pl.ds(0, DC)], 10)

    def untranspose_x(dst, c0):
        for r in range(S // 128):
            xt = ctxa[0:DM, c0 + r * 128:c0 + (r + 1) * 128].astype(F32)
            dst[r * 128:(r + 1) * 128, :] = xt.T.astype(BF)

    def relayout(raw, w2):
        for g in range(2):
            w = raw[:, g * 16:(g + 1) * 16, :].reshape(DM, 2048)
            w2[:, g * 2048:(g + 1) * 2048] = pltpu.bitcast(w, jnp.uint32)

    RB = 512
    c_bx.start()
    c_bwk.start()
    c_bx.wait()
    c_bwv.start()
    untranspose_x(bx, 0)
    c_bwk.wait()
    c_bwq.start()
    for c in (*c_bwo, c_ax, c_ckv):
        c.start()
    relayout(raw0, wk2)
    c_awq.start()

    def proj(w2, dst):
        def body(r, carry):
            rows = pl.ds(pl.multiple_of(r * RB, RB), RB)
            xr = bx[rows, :]
            for g in range(4):
                cols = slice(g * 1024, (g + 1) * 1024)
                dst[rows, cols] = _dot(xr, _w(w2, cols=cols)).astype(BF)
            return carry
        lax.fori_loop(0, S // RB, body, 0)

    with jax.named_scope('ph1_k'):
        proj(wk2, kx)
    c_bwv.wait()
    relayout(raw1, wv2)
    c_awk.start()
    with jax.named_scope('ph1_v'):
        proj(wv2, vx)
    c_bwq.wait()
    relayout(raw2, wq2)
    c_awv.start()
    for c in c_bwo:
        c.wait()
    for h in range(H):
        wt = ctxa[1024:1024 + DM, h * DH:(h + 1) * DH].astype(F32).T.astype(BF)
        bwo[h * 64:(h + 1) * 64, :] = pltpu.bitcast(wt, jnp.uint32)
    for c in c_awo:
        c.start()
    c_ax.wait()
    untranspose_x(ax, S)
    c_ckv.wait(); c_awq.wait(); c_awk.wait(); c_awv.wait()

    G = 4
    gr = lax.broadcasted_iota(jnp.int32, (G * MEM, G * (SEG + MEM)), 0) // MEM
    gc = lax.broadcasted_iota(jnp.int32, (G * MEM, G * (SEG + MEM)), 1)
    gvis = jnp.where(gc < G * SEG, gc // SEG, (gc - G * SEG) // MEM) == gr

    def mem_step(mem, s):
        q = _dot(mem, _w(wq2)) * QSCALE
        k = _dot(mem, _w(wk2))
        v = _dot(mem, _w(wv2))
        rows = pl.ds(pl.multiple_of(s * SEG, SEG), SEG)
        scs, vvs = [], []
        for g in range(H // G):
            cs = [slice(h * DH, (h + 1) * DH) for h in range(g * G, (g + 1) * G)]
            qg = jnp.concatenate([q[:, c] for c in cs], axis=0).astype(BF)
            km = jnp.concatenate([k[:, c] for c in cs], axis=0).astype(BF)
            kk = jnp.concatenate([kx[rows, c] for c in cs] + [km], axis=0)
            scs.append(jnp.where(gvis, _dot_nt(qg, kk), NEG))
        sc = jnp.concatenate(scs, axis=0)
        m = jnp.max(sc, axis=1, keepdims=True)
        p = jnp.exp2(sc - m)
        r = _recip(jnp.sum(p, axis=1, keepdims=True))
        p = p.astype(BF)
        ctx = []
        for g in range(H // G):
            cs = [slice(h * DH, (h + 1) * DH) for h in range(g * G, (g + 1) * G)]
            vm = jnp.concatenate([v[:, c] for c in cs], axis=0).astype(BF)
            vv = jnp.concatenate([vx[rows, c] for c in cs] + [vm], axis=0)
            gs = slice(g * G * MEM, (g + 1) * G * MEM)
            o = _dot(p[gs], vv) * r[gs]
            ctx += [o[j * MEM:(j + 1) * MEM] for j in range(G)]
        ctx = jnp.concatenate(ctx, axis=1).astype(BF)
        return _dot(ctx, _w(bwo)).astype(BF), k, v

    def rec_pair(p, mem):
        mem1, k0, v0 = mem_step(mem, 2 * p)
        mem2, k1, v1 = mem_step(mem1, 2 * p + 1)
        prow = pl.ds(pl.multiple_of(p * 16, 16), 16)
        kmem[prow, :] = jnp.concatenate([k0, k1], axis=0).astype(BF)
        vmem[prow, :] = jnp.concatenate([v0, v1], axis=0).astype(BF)
        return mem2

    with jax.named_scope('rec'):
        lax.fori_loop(0, NSEG // 2, rec_pair, mem0_ref[...])

    BQ = 256
    tri = (lax.broadcasted_iota(jnp.int32, (BQ, BQ), 1) <= lax.broadcasted_iota(jnp.int32, (BQ, BQ), 0))

    def head_pair(raw, rows, i):
        u = raw.bitcast(jnp.uint32)[0:rows, pl.ds(i, 1), :].reshape(rows, DH)
        lo = pltpu.bitcast(u << 16, F32).astype(BF)
        hi = pltpu.bitcast(u & jnp.uint32(0xFFFF0000), F32).astype(BF)
        return lo, hi

    def a_pair(i2, carry):
        wq = head_pair(raw0, DM, i2)
        wk = head_pair(raw1, DC, i2)
        wv = head_pair(raw2, DC, i2)
        NB = S // BQ

        def project(e):
            q = (_dot(ax[...], wq[e]) * QSCALE).astype(BF)
            k = _dot(ckv[...], wk[e]).astype(BF)
            v = _dot(ckv[...], wv[e]).astype(BF)
            return q, k, v

        def scores(qkv, i):
            q, k, _ = qkv
            r0 = i * BQ
            qi = q[r0:r0 + BQ]
            sc = jnp.where(tri, _dot_nt(qi, k[r0:r0 + BQ]), NEG)
            if i > 0:
                sc = jnp.concatenate([_dot_nt(qi, k[0:r0]), sc], axis=1)
            return sc

        def finish(qkv, e, i, sc):
            cols = pl.ds(pl.multiple_of(i2 * 2 * DH + e * DH, DH), DH)
            r0 = i * BQ
            m = jnp.max(sc, axis=1, keepdims=True)
            p = jnp.exp2(sc - m)
            l = jnp.sum(p, axis=1, keepdims=True)
            o = _dot(p.astype(BF), qkv[2][0:r0 + BQ])
            ctxa[r0:r0 + BQ, cols] = (o * _recip(l)).astype(BF)

        items = [(e, i) for e in range(2) for i in range(NB)]
        qkvs = {0: project(0)}
        sc = scores(qkvs[0], 0)
        for n, (e, i) in enumerate(items):
            nxt = None
            if n + 1 < len(items):
                e1, i1 = items[n + 1]
                if e1 not in qkvs:
                    qkvs[e1] = project(e1)
                nxt = scores(qkvs[e1], i1)
            finish(qkvs[e], e, i, sc)
            sc = nxt
        return carry
    with jax.named_scope('a_attn'):
        lax.fori_loop(0, H // 2, a_pair, 0)

    for c in c_awo:
        c.wait()

    def a_out(r, carry):
        rows = pl.ds(pl.multiple_of(r * RB, RB), RB)
        o_ref[rows, 0:DM] = _dot_nt(ctxa[rows, :], awo[...]).astype(BF)
        return carry
    with jax.named_scope('a_out'):
        lax.fori_loop(0, S // RB, a_out, 0)

    T = 4
    ri = lax.broadcasted_iota(jnp.int32, (T * SEG, T * (SEG + MEM)), 0)
    ci = lax.broadcasted_iota(jnp.int32, (T * SEG, T * (SEG + MEM)), 1)
    xkey = ci < T * SEG
    cseg = jnp.where(xkey, ci // SEG, (ci - T * SEG) // MEM)
    vis = (cseg == ri // SEG) & (jnp.where(xkey, ci, 0) <= ri)

    def b_head(h, carry):
        cols = pl.ds(pl.multiple_of(h * DH, DH), DH)
        q = (_dot(bx[...], _w(wq2, cols=cols)) * QSCALE).astype(BF)
        scs = []
        for t in range(NSEG // T):
            xr = slice(t * T * SEG, (t + 1) * T * SEG)
            mr = slice(t * T * MEM, (t + 1) * T * MEM)
            kk = jnp.concatenate([kx[xr, cols], kmem[mr, cols]], axis=0)
            scs.append(jnp.where(vis, _dot_nt(q[xr], kk), NEG))
        sc = jnp.concatenate(scs, axis=0)
        m = jnp.max(sc, axis=1, keepdims=True)
        p = jnp.exp2(sc - m)
        r = _recip(jnp.sum(p, axis=1, keepdims=True))
        p = p.astype(BF)
        for t in range(NSEG // T):
            xr = slice(t * T * SEG, (t + 1) * T * SEG)
            mr = slice(t * T * MEM, (t + 1) * T * MEM)
            vv = jnp.concatenate([vx[xr, cols], vmem[mr, cols]], axis=0)
            ctxa[xr, cols] = (_dot(p[xr], vv) * r[xr]).astype(BF)
        return carry
    with jax.named_scope('b_attn'):
        lax.fori_loop(0, H, b_head, 0)

    def b_out(r, carry):
        rows = pl.ds(pl.multiple_of(r * RB, RB), RB)
        o_ref[rows, DM:2 * DM] = _dot(ctxa[rows, :], _w(bwo)).astype(BF)
        return carry
    with jax.named_scope('b_out'):
        lax.fori_loop(0, S // RB, b_out, 0)


@jax.jit
def _run(A_x, A_c_kv, A_w_q, A_w_uk, A_w_uv, A_w_o, B_x, B_mem0, B_Wq, B_Wk, B_Wv, B_Wo):
    any_spec = pl.BlockSpec(memory_space=pl.ANY)
    vm = pltpu.VMEM
    out = pl.pallas_call(
        _kernel,
        out_shape=jax.ShapeDtypeStruct((S, 2 * DM), BF),
        in_specs=[any_spec] * 7 + [pl.BlockSpec(memory_space=pltpu.VMEM)] + [any_spec] * 4,
        out_specs=pl.BlockSpec(memory_space=pltpu.VMEM),
        scratch_shapes=[
            vm((S, DM), BF), vm((S, DC), BF), vm((S, DM), BF),
            vm((DM, H, DH), BF), vm((DM, H, DH), BF), vm((DM, H, DH), BF),
            vm((DM, HD), BF), vm((HD // 2, DM), jnp.uint32),
            vm((DM // 2, HD), jnp.uint32), vm((DM // 2, HD), jnp.uint32), vm((DM // 2, HD), jnp.uint32),
            vm((S, HD), BF), vm((S, HD), BF),
            vm((NSEG * MEM, HD), BF), vm((NSEG * MEM, HD), BF),
            vm((S, HD), BF),
            pltpu.SemaphoreType.DMA((11,)),
            pltpu.SemaphoreType.DMA((2 * H,)),
        ],
        compiler_params=pltpu.CompilerParams(vmem_limit_bytes=126 * 2 ** 20),
    )(A_x.reshape(S, DM).T, A_c_kv.reshape(S, DC), A_w_q, A_w_uk, A_w_uv, jnp.transpose(A_w_o, (0, 2, 1)),
      B_x.reshape(S, DM).T, B_mem0.reshape(MEM, DM), B_Wq, B_Wk, B_Wv, jnp.transpose(B_Wo, (0, 2, 1)))
    return out.reshape(1, S, 2 * DM)


def pallas_concat_heads__compressed_kv_cla__memory_aug_recurrent_mem_tr__prompt_kernel(
        A_x, A_c_kv, A_w_q, A_w_uk, A_w_uv, A_w_o, B_x, B_mem0, B_Wq, B_Wk, B_Wv, B_Wo, B_seg_len=SEG):
    del B_seg_len
    return _run(A_x, A_c_kv, A_w_q, A_w_uk, A_w_uv, A_w_o, B_x, B_mem0, B_Wq, B_Wk, B_Wv, B_Wo)
```

```python
import functools
import math

import jax
import jax.numpy as jnp
from jax import lax
import jax.experimental.pallas as pl
import jax.experimental.pallas.tpu as pltpu

S = 2048
DM = 576
DC = 512
H = 32
DH = 128
HD = H * DH
MEM = 8
SEG = 32
NSEG = S // SEG
NEG = -1e9
LOG2E = math.log2(math.e)
QSCALE = DH ** -0.5 * LOG2E

BF = jnp.bfloat16
F32 = jnp.float32
NT = (((1,), (1,)), ((), ()))


def _dot(a, b):
    return jnp.dot(a, b, preferred_element_type=F32)


def _dot_nt(a, b):
    return lax.dot_general(a, b, NT, preferred_element_type=F32)


def _recip(l):
    r = pl.reciprocal(l, approx=True)
    return r * (2.0 - l * r)


def _w(ref, rows=slice(None), cols=slice(None)):
    return pltpu.bitcast(ref[rows, cols], BF)


def _kernel(ax_h, ckv_h, awq_h, awk_h, awv_h, awo_h, bx_h, mem0_ref, bwq_h, bwk_h, bwv_h, bwo_h,
            o_hbm,
            ax, ckv, bx, raw0, raw1, raw2, awo, bwo, wq2, wk2, wv2, kx, vx, kmem, vmem, ctxa, o_ref, sems, wsems, osems):
    def cp(src, dst, i):
        return pltpu.make_async_copy(src, dst, sems.at[i])

    c_bx = cp(bx_h, ctxa.at[0:DM, 0:S], 0)
    c_bwk = cp(bwk_h, raw0, 1)
    c_bwv = cp(bwv_h, raw1, 2)
    c_bwq = cp(bwq_h, raw2, 3)
    c_bwo = [pltpu.make_async_copy(bwo_h.at[h], ctxa.at[1024:1024 + DM, h * DH:(h + 1) * DH], wsems.at[h])
             for h in range(H)]
    c_ax = cp(ax_h, ctxa.at[0:DM, S:2 * S], 5)
    c_ckv = cp(ckv_h, ckv, 6)
    c_awo = [pltpu.make_async_copy(awo_h.at[h], awo.at[:, h * DH:(h + 1) * DH], wsems.at[H + h])
             for h in range(H)]
    c_awq = cp(awq_h, raw0, 8)
    c_awk = cp(awk_h, raw1.at[pl.ds(0, DC)], 9)
    c_awv = cp(awv_h, raw2.at[pl.ds(0, DC)], 10)

    def untranspose_x(dst, c0):
        for r in range(S // 128):
            xt = ctxa[0:DM, c0 + r * 128:c0 + (r + 1) * 128].astype(F32)
            dst[r * 128:(r + 1) * 128, :] = xt.T.astype(BF)

    def relayout(raw, w2, r=None):
        n = DM // 4
        for q4 in (range(4) if r is None else (r,)):
            src = pl.ds(pl.multiple_of(q4 * n, 16), n)
            dst = pl.ds(pl.multiple_of(q4 * (n // 2), 8), n // 2)
            for g in range(2):
                w = raw[src, g * 16:(g + 1) * 16, :].reshape(n, 2048)
                w2[dst, g * 2048:(g + 1) * 2048] = pltpu.bitcast(w, jnp.uint32)

    RB = 512
    c_bx.start()
    c_bwk.start()
    c_bx.wait()
    c_bwv.start()
    untranspose_x(bx, 0)
    c_bwk.wait()
    c_bwq.start()
    for c in (*c_bwo, c_ax, c_ckv):
        c.start()
    relayout(raw0, wk2)
    c_awq.start()

    def proj(w2, dst, extra):
        def body(r, carry):
            rows = pl.ds(pl.multiple_of(r * RB, RB), RB)
            xr = bx[rows, :]
            for g in range(4):
                cols = slice(g * 1024, (g + 1) * 1024)
                dst[rows, cols] = _dot(xr, _w(w2, cols=cols)).astype(BF)
                extra(r, g)
            return carry
        lax.fori_loop(0, S // RB, body, 0)

    def extra_k(r, g):
        if g == 0:
            relayout(raw1, wv2, r)

    def extra_v(r, g):
        if g == 0:
            relayout(raw2, wq2, r)
        elif g == 1:
            for j in range(H // 4):
                h = r * (H // 4) + j
                hc = pl.ds(pl.multiple_of(h * DH, DH), DH)
                wt = ctxa[1024:1024 + DM, hc].astype(F32).T.astype(BF)
                bwo[pl.ds(pl.multiple_of(h * 64, 64), 64), :] = pltpu.bitcast(wt, jnp.uint32)
        elif g == 2:
            for j in range(4):
                t = r * 4 + j
                xt = ctxa[0:DM, pl.ds(pl.multiple_of(S + t * 128, 128), 128)].astype(F32)
                ax[pl.ds(pl.multiple_of(t * 128, 128), 128), :] = xt.T.astype(BF)

    c_bwv.wait()
    with jax.named_scope('ph1_k'):
        proj(wk2, kx, extra_k)
    c_awk.start()
    c_bwq.wait()
    for c in c_bwo:
        c.wait()
    c_ax.wait()
    with jax.named_scope('ph1_v'):
        proj(wv2, vx, extra_v)
    c_awv.start()
    for c in c_awo:
        c.start()
    c_ckv.wait(); c_awq.wait(); c_awk.wait()

    G = 4
    gr = lax.broadcasted_iota(jnp.int32, (G * MEM, G * (SEG + MEM)), 0) // MEM
    gc = lax.broadcasted_iota(jnp.int32, (G * MEM, G * (SEG + MEM)), 1)
    gvis = jnp.where(gc < G * SEG, gc // SEG, (gc - G * SEG) // MEM) == gr

    def mem_step(mem, s):
        q = _dot(mem, _w(wq2)) * QSCALE
        k = _dot(mem, _w(wk2))
        v = _dot(mem, _w(wv2))
        rows = pl.ds(pl.multiple_of(s * SEG, SEG), SEG)
        scs, vvs = [], []
        for g in range(H // G):
            cs = [slice(h * DH, (h + 1) * DH) for h in range(g * G, (g + 1) * G)]
            qg = jnp.concatenate([q[:, c] for c in cs], axis=0).astype(BF)
            km = jnp.concatenate([k[:, c] for c in cs], axis=0).astype(BF)
            kk = jnp.concatenate([kx[rows, c] for c in cs] + [km], axis=0)
            scs.append(jnp.where(gvis, _dot_nt(qg, kk), NEG))
        sc = jnp.concatenate(scs, axis=0)
        m = jnp.max(sc, axis=1, keepdims=True)
        p = jnp.exp2(sc - m)
        r = _recip(jnp.sum(p, axis=1, keepdims=True))
        p = p.astype(BF)
        ctx = []
        for g in range(H // G):
            cs = [slice(h * DH, (h + 1) * DH) for h in range(g * G, (g + 1) * G)]
            vm = jnp.concatenate([v[:, c] for c in cs], axis=0).astype(BF)
            vv = jnp.concatenate([vx[rows, c] for c in cs] + [vm], axis=0)
            gs = slice(g * G * MEM, (g + 1) * G * MEM)
            o = _dot(p[gs], vv) * r[gs]
            ctx += [o[j * MEM:(j + 1) * MEM] for j in range(G)]
        ctx = jnp.concatenate(ctx, axis=1).astype(BF)
        return _dot(ctx, _w(bwo)).astype(BF), k, v

    def rec_pair(p, mem):
        mem1, k0, v0 = mem_step(mem, 2 * p)
        mem2, k1, v1 = mem_step(mem1, 2 * p + 1)
        prow = pl.ds(pl.multiple_of(p * 16, 16), 16)
        kmem[prow, :] = jnp.concatenate([k0, k1], axis=0).astype(BF)
        vmem[prow, :] = jnp.concatenate([v0, v1], axis=0).astype(BF)
        return mem2

    with jax.named_scope('rec'):
        lax.fori_loop(0, NSEG // 2, rec_pair, mem0_ref[...])

    c_awv.wait()
    BQ = 128
    tri = (lax.broadcasted_iota(jnp.int32, (BQ, BQ), 1) <= lax.broadcasted_iota(jnp.int32, (BQ, BQ), 0))

    def head_pair(raw, rows, i):
        u = raw.bitcast(jnp.uint32)[0:rows, pl.ds(i, 1), :].reshape(rows, DH)
        lo = pltpu.bitcast(u << 16, F32).astype(BF)
        hi = pltpu.bitcast(u & jnp.uint32(0xFFFF0000), F32).astype(BF)
        return lo, hi

    def a_pair(i2, carry):
        wq = head_pair(raw0, DM, i2)
        wk = head_pair(raw1, DC, i2)
        wv = head_pair(raw2, DC, i2)
        NB = S // BQ

        q2 = (_dot(ax[...], jnp.concatenate(wq, axis=1)) * QSCALE).astype(BF)
        kv = _dot(ckv[...], jnp.concatenate([wk[0], wv[0], wk[1], wv[1]], axis=1)).astype(BF)

        def project(e):
            return q2[:, e * DH:(e + 1) * DH], kv[:, 2 * e * DH:(2 * e + 1) * DH], kv[:, (2 * e + 1) * DH:(2 * e + 2) * DH]

        def scores(qkv, i):
            q, k, _ = qkv
            r0 = i * BQ
            qi = q[r0:r0 + BQ]
            sc = jnp.where(tri, _dot_nt(qi, k[r0:r0 + BQ]), NEG)
            if i > 0:
                sc = jnp.concatenate([_dot_nt(qi, k[0:r0]), sc], axis=1)
            return sc

        def finish(qkv, e, i, sc):
            cols = pl.ds(pl.multiple_of(i2 * 2 * DH + e * DH, DH), DH)
            r0 = i * BQ
            m = jnp.max(sc, axis=1, keepdims=True)
            p = jnp.exp2(sc - m)
            l = jnp.sum(p, axis=1, keepdims=True)
            o = _dot(p.astype(BF), qkv[2][0:r0 + BQ])
            ctxa[r0:r0 + BQ, cols] = (o * _recip(l)).astype(BF)

        items = [(e, i) for e in range(2) for i in range(NB)]
        qkvs = {0: project(0)}
        sc = scores(qkvs[0], 0)
        for n, (e, i) in enumerate(items):
            nxt = None
            if n + 1 < len(items):
                e1, i1 = items[n + 1]
                if e1 not in qkvs:
                    qkvs[e1] = project(e1)
                nxt = scores(qkvs[e1], i1)
            finish(qkvs[e], e, i, sc)
            sc = nxt
        return carry
    with jax.named_scope('a_attn'):
        lax.fori_loop(0, H // 2, a_pair, 0)

    for c in c_awo:
        c.wait()

    def a_out(r, carry):
        rows = pl.ds(pl.multiple_of(r * RB, RB), RB)
        o_ref[rows, 0:DM] = _dot_nt(ctxa[rows, :], awo[...]).astype(BF)
        return carry
    with jax.named_scope('a_out'):
        lax.fori_loop(0, S // RB, a_out, 0)

    T = 2
    ri = lax.broadcasted_iota(jnp.int32, (T * SEG, T * (SEG + MEM)), 0)
    ci = lax.broadcasted_iota(jnp.int32, (T * SEG, T * (SEG + MEM)), 1)
    xkey = ci < T * SEG
    cseg = jnp.where(xkey, ci // SEG, (ci - T * SEG) // MEM)
    vis = (cseg == ri // SEG) & (jnp.where(xkey, ci, 0) <= ri)

    def b_head(h, carry):
        cols = pl.ds(pl.multiple_of(h * DH, DH), DH)
        q = (_dot(bx[...], _w(wq2, cols=cols)) * QSCALE).astype(BF)
        scs = []
        for t in range(NSEG // T):
            xr = slice(t * T * SEG, (t + 1) * T * SEG)
            mr = slice(t * T * MEM, (t + 1) * T * MEM)
            kk = jnp.concatenate([kx[xr, cols], kmem[mr, cols]], axis=0)
            scs.append(jnp.where(vis, _dot_nt(q[xr], kk), NEG))
        sc = jnp.concatenate(scs, axis=0)
        m = jnp.max(sc, axis=1, keepdims=True)
        p = jnp.exp2(sc - m)
        r = _recip(jnp.sum(p, axis=1, keepdims=True))
        p = p.astype(BF)
        for t in range(NSEG // T):
            xr = slice(t * T * SEG, (t + 1) * T * SEG)
            mr = slice(t * T * MEM, (t + 1) * T * MEM)
            vv = jnp.concatenate([vx[xr, cols], vmem[mr, cols]], axis=0)
            ctxa[xr, cols] = (_dot(p[xr], vv) * r[xr]).astype(BF)
        return carry
    with jax.named_scope('b_attn'):
        lax.fori_loop(0, H, b_head, 0)

    def b_out(r, carry):
        rows = pl.ds(pl.multiple_of(r * RB, RB), RB)
        o_ref[rows, DM:2 * DM] = _dot(ctxa[rows, :], _w(bwo)).astype(BF)
        pltpu.make_async_copy(o_ref.at[rows], o_hbm.at[rows], osems.at[r]).start()
        return carry
    with jax.named_scope('b_out'):
        lax.fori_loop(0, S // RB, b_out, 0)
    for r in range(S // RB):
        rows = pl.ds(r * RB, RB)
        pltpu.make_async_copy(o_ref.at[rows], o_hbm.at[rows], osems.at[r]).wait()


@jax.jit
def _run(A_x, A_c_kv, A_w_q, A_w_uk, A_w_uv, A_w_o, B_x, B_mem0, B_Wq, B_Wk, B_Wv, B_Wo):
    any_spec = pl.BlockSpec(memory_space=pl.ANY)
    vm = pltpu.VMEM
    out = pl.pallas_call(
        _kernel,
        out_shape=jax.ShapeDtypeStruct((S, 2 * DM), BF),
        in_specs=[any_spec] * 7 + [pl.BlockSpec(memory_space=pltpu.VMEM)] + [any_spec] * 4,
        out_specs=any_spec,
        scratch_shapes=[
            vm((S, DM), BF), vm((S, DC), BF), vm((S, DM), BF),
            vm((DM, H, DH), BF), vm((DM, H, DH), BF), vm((DM, H, DH), BF),
            vm((DM, HD), BF), vm((HD // 2, DM), jnp.uint32),
            vm((DM // 2, HD), jnp.uint32), vm((DM // 2, HD), jnp.uint32), vm((DM // 2, HD), jnp.uint32),
            vm((S, HD), BF), vm((S, HD), BF),
            vm((NSEG * MEM, HD), BF), vm((NSEG * MEM, HD), BF),
            vm((S, HD), BF),
            vm((S, 2 * DM), BF),
            pltpu.SemaphoreType.DMA((11,)),
            pltpu.SemaphoreType.DMA((2 * H,)),
            pltpu.SemaphoreType.DMA((4,)),
        ],
        compiler_params=pltpu.CompilerParams(vmem_limit_bytes=126 * 2 ** 20),
    )(A_x.reshape(S, DM).T, A_c_kv.reshape(S, DC), A_w_q, A_w_uk, A_w_uv, jnp.transpose(A_w_o, (0, 2, 1)),
      B_x.reshape(S, DM).T, B_mem0.reshape(MEM, DM), B_Wq, B_Wk, B_Wv, jnp.transpose(B_Wo, (0, 2, 1)))
    return out.reshape(1, S, 2 * DM)


def pallas_concat_heads__compressed_kv_cla__memory_aug_recurrent_mem_tr__prompt_kernel(
        A_x, A_c_kv, A_w_q, A_w_uk, A_w_uv, A_w_o, B_x, B_mem0, B_Wq, B_Wk, B_Wv, B_Wo, B_seg_len=SEG):
    del B_seg_len
    return _run(A_x, A_c_kv, A_w_q, A_w_uk, A_w_uv, A_w_o, B_x, B_mem0, B_Wq, B_Wk, B_Wv, B_Wo)
```

```python
import functools
import math

import jax
import jax.numpy as jnp
from jax import lax
import jax.experimental.pallas as pl
import jax.experimental.pallas.tpu as pltpu

S = 2048
DM = 576
DC = 512
H = 32
DH = 128
HD = H * DH
MEM = 8
SEG = 32
NSEG = S // SEG
NEG = -1e9
LOG2E = math.log2(math.e)
QSCALE = DH ** -0.5 * LOG2E

BF = jnp.bfloat16
F32 = jnp.float32
NT = (((1,), (1,)), ((), ()))


def _dot(a, b):
    return jnp.dot(a, b, preferred_element_type=F32)


def _dot_nt(a, b):
    return lax.dot_general(a, b, NT, preferred_element_type=F32)


def _recip(l):
    r = pl.reciprocal(l, approx=True)
    return r * (2.0 - l * r)


def _w(ref, rows=slice(None), cols=slice(None)):
    return pltpu.bitcast(ref[rows, cols], BF)


def _kernel(ax_h, ckv_h, awq_h, awk_h, awv_h, awo_h, bx_h, mem0_ref, bwq_h, bwk_h, bwv_h, bwo_h,
            o_hbm,
            ax, ckv, bx, raw0, raw1, raw2, awo, bwo, wq2, wk2, wv2, kx, vx, kmem, vmem, ctxa, o_ref, bwot, sems, wsems, osems):
    def cp(src, dst, i):
        return pltpu.make_async_copy(src, dst, sems.at[i])

    c_bx = cp(bx_h, ctxa.at[0:DM, 0:S], 0)
    c_bwk = cp(bwk_h, raw0, 1)
    c_bwv = cp(bwv_h, raw1, 2)
    c_bwq = cp(bwq_h, raw2, 3)
    c_bwo = [pltpu.make_async_copy(bwo_h.at[h], ctxa.at[1024:1024 + DM, h * DH:(h + 1) * DH], wsems.at[h])
             for h in range(H)]
    c_ax = cp(ax_h, ctxa.at[0:DM, S:2 * S], 5)
    c_ckv = cp(ckv_h, ckv, 6)
    c_awo = [pltpu.make_async_copy(awo_h.at[h], awo.at[:, h * DH:(h + 1) * DH], wsems.at[H + h])
             for h in range(H)]
    c_bwot = [pltpu.make_async_copy(bwo_h.at[h], bwot.at[:, h * DH:(h + 1) * DH], wsems.at[h])
              for h in range(H)]
    c_awq = cp(awq_h, raw0, 8)
    c_awk = cp(awk_h, raw1.at[pl.ds(0, DC)], 9)
    c_awv = cp(awv_h, raw2.at[pl.ds(0, DC)], 10)

    def untranspose_x(dst, c0):
        for r in range(S // 128):
            xt = ctxa[0:DM, c0 + r * 128:c0 + (r + 1) * 128].astype(F32)
            dst[r * 128:(r + 1) * 128, :] = xt.T.astype(BF)

    def relayout(raw, w2, r=None):
        n = DM // 4
        for q4 in (range(4) if r is None else (r,)):
            src = pl.ds(pl.multiple_of(q4 * n, 16), n)
            dst = pl.ds(pl.multiple_of(q4 * (n // 2), 8), n // 2)
            for g in range(2):
                w = raw[src, g * 16:(g + 1) * 16, :].reshape(n, 2048)
                w2[dst, g * 2048:(g + 1) * 2048] = pltpu.bitcast(w, jnp.uint32)

    RB = 512
    c_bx.start()
    c_bwk.start()
    c_bx.wait()
    c_bwv.start()
    untranspose_x(bx, 0)
    c_bwk.wait()
    c_bwq.start()
    for c in (*c_bwo, c_ax, c_ckv):
        c.start()
    relayout(raw0, wk2)
    c_awq.start()

    def proj(w2, dst, extra):
        def body(r, carry):
            rows = pl.ds(pl.multiple_of(r * RB, RB), RB)
            xr = bx[rows, :]
            for g in range(4):
                cols = slice(g * 1024, (g + 1) * 1024)
                dst[rows, cols] = _dot(xr, _w(w2, cols=cols)).astype(BF)
                extra(r, g)
            return carry
        lax.fori_loop(0, S // RB, body, 0)

    def extra_k(r, g):
        if g == 0:
            relayout(raw1, wv2, r)

    def extra_v(r, g):
        if g == 0:
            relayout(raw2, wq2, r)
        elif g == 1:
            for j in range(H // 4):
                h = r * (H // 4) + j
                hc = pl.ds(pl.multiple_of(h * DH, DH), DH)
                wt = ctxa[1024:1024 + DM, hc].astype(F32).T.astype(BF)
                bwo[pl.ds(pl.multiple_of(h * 64, 64), 64), :] = pltpu.bitcast(wt, jnp.uint32)
        elif g == 2:
            for j in range(4):
                t = r * 4 + j
                xt = ctxa[0:DM, pl.ds(pl.multiple_of(S + t * 128, 128), 128)].astype(F32)
                ax[pl.ds(pl.multiple_of(t * 128, 128), 128), :] = xt.T.astype(BF)

    c_bwv.wait()
    with jax.named_scope('ph1_k'):
        proj(wk2, kx, extra_k)
    c_awk.start()
    c_bwq.wait()
    for c in c_bwo:
        c.wait()
    c_ax.wait()
    with jax.named_scope('ph1_v'):
        proj(wv2, vx, extra_v)
    c_awv.start()
    for c in (*c_awo, *c_bwot):
        c.start()
    c_ckv.wait(); c_awq.wait(); c_awk.wait()

    G = 4
    gr = lax.broadcasted_iota(jnp.int32, (G * MEM, G * (SEG + MEM)), 0) // MEM
    gc = lax.broadcasted_iota(jnp.int32, (G * MEM, G * (SEG + MEM)), 1)
    gvis = jnp.where(gc < G * SEG, gc // SEG, (gc - G * SEG) // MEM) == gr

    def mem_step(mem, s):
        q = _dot(mem, _w(wq2)) * QSCALE
        k = _dot(mem, _w(wk2))
        v = _dot(mem, _w(wv2))
        rows = pl.ds(pl.multiple_of(s * SEG, SEG), SEG)
        scs, vvs = [], []
        for g in range(H // G):
            cs = [slice(h * DH, (h + 1) * DH) for h in range(g * G, (g + 1) * G)]
            qg = jnp.concatenate([q[:, c] for c in cs], axis=0).astype(BF)
            km = jnp.concatenate([k[:, c] for c in cs], axis=0).astype(BF)
            kk = jnp.concatenate([kx[rows, c] for c in cs] + [km], axis=0)
            scs.append(jnp.where(gvis, _dot_nt(qg, kk), NEG))
        sc = jnp.concatenate(scs, axis=0)
        m = jnp.max(sc, axis=1, keepdims=True)
        p = jnp.exp2(sc - m)
        r = _recip(jnp.sum(p, axis=1, keepdims=True))
        p = p.astype(BF)
        ctx = []
        for g in range(H // G):
            cs = [slice(h * DH, (h + 1) * DH) for h in range(g * G, (g + 1) * G)]
            vm = jnp.concatenate([v[:, c] for c in cs], axis=0).astype(BF)
            vv = jnp.concatenate([vx[rows, c] for c in cs] + [vm], axis=0)
            gs = slice(g * G * MEM, (g + 1) * G * MEM)
            o = _dot(p[gs], vv) * r[gs]
            ctx += [o[j * MEM:(j + 1) * MEM] for j in range(G)]
        ctx = jnp.concatenate(ctx, axis=1).astype(BF)
        return _dot(ctx, _w(bwo)).astype(BF), k, v

    def rec_pair(p, mem):
        mem1, k0, v0 = mem_step(mem, 2 * p)
        mem2, k1, v1 = mem_step(mem1, 2 * p + 1)
        prow = pl.ds(pl.multiple_of(p * 16, 16), 16)
        kmem[prow, :] = jnp.concatenate([k0, k1], axis=0).astype(BF)
        vmem[prow, :] = jnp.concatenate([v0, v1], axis=0).astype(BF)
        return mem2

    with jax.named_scope('rec'):
        lax.fori_loop(0, NSEG // 2, rec_pair, mem0_ref[...])

    c_awv.wait()
    BQ = 128
    tri = (lax.broadcasted_iota(jnp.int32, (BQ, BQ), 1) <= lax.broadcasted_iota(jnp.int32, (BQ, BQ), 0))

    def head_pair(raw, rows, i):
        u = raw.bitcast(jnp.uint32)[0:rows, pl.ds(i, 1), :].reshape(rows, DH)
        lo = pltpu.bitcast(u << 16, F32).astype(BF)
        hi = pltpu.bitcast(u & jnp.uint32(0xFFFF0000), F32).astype(BF)
        return lo, hi

    def a_pair(i2, carry):
        wq = head_pair(raw0, DM, i2)
        wk = head_pair(raw1, DC, i2)
        wv = head_pair(raw2, DC, i2)
        NB = S // BQ

        q2 = (_dot(ax[...], jnp.concatenate(wq, axis=1)) * QSCALE).astype(BF)
        kv = _dot(ckv[...], jnp.concatenate([wk[0], wv[0], wk[1], wv[1]], axis=1)).astype(BF)

        def project(e):
            return q2[:, e * DH:(e + 1) * DH], kv[:, 2 * e * DH:(2 * e + 1) * DH], kv[:, (2 * e + 1) * DH:(2 * e + 2) * DH]

        def scores(qkv, i):
            q, k, _ = qkv
            r0 = i * BQ
            qi = q[r0:r0 + BQ]
            sc = jnp.where(tri, _dot_nt(qi, k[r0:r0 + BQ]), NEG)
            if i > 0:
                sc = jnp.concatenate([_dot_nt(qi, k[0:r0]), sc], axis=1)
            return sc

        def finish(qkv, e, i, sc):
            cols = pl.ds(pl.multiple_of(i2 * 2 * DH + e * DH, DH), DH)
            r0 = i * BQ
            m = jnp.max(sc, axis=1, keepdims=True)
            p = jnp.exp2(sc - m)
            l = jnp.sum(p, axis=1, keepdims=True)
            o = _dot(p.astype(BF), qkv[2][0:r0 + BQ])
            ctxa[r0:r0 + BQ, cols] = (o * _recip(l)).astype(BF)

        items = [(e, i) for e in range(2) for i in range(NB)]
        qkvs = {0: project(0)}
        sc = scores(qkvs[0], 0)
        for n, (e, i) in enumerate(items):
            nxt = None
            if n + 1 < len(items):
                e1, i1 = items[n + 1]
                if e1 not in qkvs:
                    qkvs[e1] = project(e1)
                nxt = scores(qkvs[e1], i1)
            finish(qkvs[e], e, i, sc)
            sc = nxt
        return carry
    with jax.named_scope('a_attn'):
        lax.fori_loop(0, H // 2, a_pair, 0)

    for c in (*c_awo, *c_bwot):
        c.wait()

    def a_out(r, carry):
        rows = pl.ds(pl.multiple_of(r * RB, RB), RB)
        o_ref[rows, 0:DM] = _dot_nt(awo[...], ctxa[rows, :]).T.astype(BF)
        return carry
    with jax.named_scope('a_out'):
        lax.fori_loop(0, S // RB, a_out, 0)

    T = 2
    ri = lax.broadcasted_iota(jnp.int32, (T * SEG, T * (SEG + MEM)), 0)
    ci = lax.broadcasted_iota(jnp.int32, (T * SEG, T * (SEG + MEM)), 1)
    xkey = ci < T * SEG
    cseg = jnp.where(xkey, ci // SEG, (ci - T * SEG) // MEM)
    vis = (cseg == ri // SEG) & (jnp.where(xkey, ci, 0) <= ri)

    def b_head(h, carry):
        cols = pl.ds(pl.multiple_of(h * DH, DH), DH)
        q = (_dot(bx[...], _w(wq2, cols=cols)) * QSCALE).astype(BF)
        scs = []
        for t in range(NSEG // T):
            xr = slice(t * T * SEG, (t + 1) * T * SEG)
            mr = slice(t * T * MEM, (t + 1) * T * MEM)
            kk = jnp.concatenate([kx[xr, cols], kmem[mr, cols]], axis=0)
            scs.append(jnp.where(vis, _dot_nt(q[xr], kk), NEG))
        sc = jnp.concatenate(scs, axis=0)
        m = jnp.max(sc, axis=1, keepdims=True)
        p = jnp.exp2(sc - m)
        r = _recip(jnp.sum(p, axis=1, keepdims=True))
        p = p.astype(BF)
        for t in range(NSEG // T):
            xr = slice(t * T * SEG, (t + 1) * T * SEG)
            mr = slice(t * T * MEM, (t + 1) * T * MEM)
            vv = jnp.concatenate([vx[xr, cols], vmem[mr, cols]], axis=0)
            ctxa[xr, cols] = (_dot(p[xr], vv) * r[xr]).astype(BF)
        return carry
    with jax.named_scope('b_attn'):
        lax.fori_loop(0, H, b_head, 0)

    def b_out(r, carry):
        rows = pl.ds(pl.multiple_of(r * RB, RB), RB)
        o_ref[rows, DM:2 * DM] = _dot_nt(bwot[...], ctxa[rows, :]).T.astype(BF)
        pltpu.make_async_copy(o_ref.at[rows], o_hbm.at[rows], osems.at[r]).start()
        return carry
    with jax.named_scope('b_out'):
        lax.fori_loop(0, S // RB, b_out, 0)
    for r in range(S // RB):
        rows = pl.ds(r * RB, RB)
        pltpu.make_async_copy(o_ref.at[rows], o_hbm.at[rows], osems.at[r]).wait()


@jax.jit
def _run(A_x, A_c_kv, A_w_q, A_w_uk, A_w_uv, A_w_o, B_x, B_mem0, B_Wq, B_Wk, B_Wv, B_Wo):
    any_spec = pl.BlockSpec(memory_space=pl.ANY)
    vm = pltpu.VMEM
    out = pl.pallas_call(
        _kernel,
        out_shape=jax.ShapeDtypeStruct((S, 2 * DM), BF),
        in_specs=[any_spec] * 7 + [pl.BlockSpec(memory_space=pltpu.VMEM)] + [any_spec] * 4,
        out_specs=any_spec,
        scratch_shapes=[
            vm((S, DM), BF), vm((S, DC), BF), vm((S, DM), BF),
            vm((DM, H, DH), BF), vm((DM, H, DH), BF), vm((DM, H, DH), BF),
            vm((DM, HD), BF), vm((HD // 2, DM), jnp.uint32),
            vm((DM // 2, HD), jnp.uint32), vm((DM // 2, HD), jnp.uint32), vm((DM // 2, HD), jnp.uint32),
            vm((S, HD), BF), vm((S, HD), BF),
            vm((NSEG * MEM, HD), BF), vm((NSEG * MEM, HD), BF),
            vm((S, HD), BF),
            vm((S, 2 * DM), BF),
            vm((DM, HD), BF),
            pltpu.SemaphoreType.DMA((11,)),
            pltpu.SemaphoreType.DMA((2 * H,)),
            pltpu.SemaphoreType.DMA((4,)),
        ],
        compiler_params=pltpu.CompilerParams(vmem_limit_bytes=126 * 2 ** 20),
    )(A_x.reshape(S, DM).T, A_c_kv.reshape(S, DC), A_w_q, A_w_uk, A_w_uv, jnp.transpose(A_w_o, (0, 2, 1)),
      B_x.reshape(S, DM).T, B_mem0.reshape(MEM, DM), B_Wq, B_Wk, B_Wv, jnp.transpose(B_Wo, (0, 2, 1)))
    return out.reshape(1, S, 2 * DM)


def pallas_concat_heads__compressed_kv_cla__memory_aug_recurrent_mem_tr__prompt_kernel(
        A_x, A_c_kv, A_w_q, A_w_uk, A_w_uv, A_w_o, B_x, B_mem0, B_Wq, B_Wk, B_Wv, B_Wo, B_seg_len=SEG):
    del B_seg_len
    return _run(A_x, A_c_kv, A_w_q, A_w_uk, A_w_uv, A_w_o, B_x, B_mem0, B_Wq, B_Wk, B_Wv, B_Wo)
```

```python
import functools
import math

import jax
import jax.numpy as jnp
from jax import lax
import jax.experimental.pallas as pl
import jax.experimental.pallas.tpu as pltpu

S = 2048
DM = 576
DC = 512
H = 32
DH = 128
HD = H * DH
MEM = 8
SEG = 32
NSEG = S // SEG
NEG = -1e9
LOG2E = math.log2(math.e)
QSCALE = DH ** -0.5 * LOG2E

BF = jnp.bfloat16
F32 = jnp.float32
NT = (((1,), (1,)), ((), ()))


def _dot(a, b):
    return jnp.dot(a, b, preferred_element_type=F32)


def _dot_nt(a, b):
    return lax.dot_general(a, b, NT, preferred_element_type=F32)


def _recip(l):
    r = pl.reciprocal(l, approx=True)
    return r * (2.0 - l * r)


def _w(ref, rows=slice(None), cols=slice(None)):
    return pltpu.bitcast(ref[rows, cols], BF)


def _kernel(ax_h, ckv_h, awq_h, awk_h, awv_h, awo_h, bx_h, mem0_ref, bwq_h, bwk_h, bwv_h, bwo_h,
            o_hbm,
            ax, ckv, bx, raw0, raw1, raw2, awo, bwo, wq2, wk2, wv2, kx, vx, kmem, vmem, ctxa, o_ref, bwot, sems, wsems, osems):
    def cp(src, dst, i):
        return pltpu.make_async_copy(src, dst, sems.at[i])

    c_bx = cp(bx_h, ctxa.at[0:DM, 0:S], 0)
    c_bwk = cp(bwk_h, raw0, 1)
    c_bwv = cp(bwv_h, raw1, 2)
    c_bwq = cp(bwq_h, raw2, 3)
    c_bwo = [pltpu.make_async_copy(bwo_h.at[h], ctxa.at[1024:1024 + DM, h * DH:(h + 1) * DH], wsems.at[h])
             for h in range(H)]
    c_ax = cp(ax_h, ctxa.at[0:DM, S:2 * S], 5)
    c_ckv = cp(ckv_h, ckv, 6)
    c_awo = [pltpu.make_async_copy(awo_h.at[h], awo.at[:, h * DH:(h + 1) * DH], wsems.at[H + h])
             for h in range(H)]
    c_bwot = [pltpu.make_async_copy(bwo_h.at[h], bwot.at[:, h * DH:(h + 1) * DH], wsems.at[h])
              for h in range(H)]
    c_awq = cp(awq_h, raw0, 8)
    c_awk = cp(awk_h, raw1.at[pl.ds(0, DC)], 9)
    c_awv = cp(awv_h, raw2.at[pl.ds(0, DC)], 10)

    def untranspose_x(dst, c0):
        for r in range(S // 128):
            xt = ctxa[0:DM, c0 + r * 128:c0 + (r + 1) * 128].astype(F32)
            dst[r * 128:(r + 1) * 128, :] = xt.T.astype(BF)

    def relayout(raw, w2, r=None):
        n = DM // 4
        for q4 in (range(4) if r is None else (r,)):
            src = pl.ds(pl.multiple_of(q4 * n, 16), n)
            dst = pl.ds(pl.multiple_of(q4 * (n // 2), 8), n // 2)
            for g in range(2):
                w = raw[src, g * 16:(g + 1) * 16, :].reshape(n, 2048)
                w2[dst, g * 2048:(g + 1) * 2048] = pltpu.bitcast(w, jnp.uint32)

    RB = 512
    c_bx.start()
    c_bwk.start()
    c_bx.wait()
    c_bwv.start()
    untranspose_x(bx, 0)
    c_bwk.wait()
    c_bwq.start()
    for c in (*c_bwo, c_ax, c_ckv):
        c.start()
    relayout(raw0, wk2)
    c_awq.start()

    def proj(w2, dst, extra):
        def body(r, carry):
            rows = pl.ds(pl.multiple_of(r * RB, RB), RB)
            xr = bx[rows, :]
            for g in range(4):
                cols = slice(g * 1024, (g + 1) * 1024)
                dst[rows, cols] = _dot(xr, _w(w2, cols=cols)).astype(BF)
                extra(r, g)
            return carry
        lax.fori_loop(0, S // RB, body, 0)

    def extra_k(r, g):
        if g == 0:
            relayout(raw1, wv2, r)

    def extra_v(r, g):
        if g == 0:
            relayout(raw2, wq2, r)
        elif g == 1:
            for j in range(H // 4):
                h = r * (H // 4) + j
                hc = pl.ds(pl.multiple_of(h * DH, DH), DH)
                wt = ctxa[1024:1024 + DM, hc].astype(F32).T.astype(BF)
                bwo[pl.ds(pl.multiple_of(h * 64, 64), 64), :] = pltpu.bitcast(wt, jnp.uint32)
        elif g == 2:
            for j in range(4):
                t = r * 4 + j
                xt = ctxa[0:DM, pl.ds(pl.multiple_of(S + t * 128, 128), 128)].astype(F32)
                ax[pl.ds(pl.multiple_of(t * 128, 128), 128), :] = xt.T.astype(BF)

    c_bwv.wait()
    with jax.named_scope('ph1_k'):
        proj(wk2, kx, extra_k)
    c_awk.start()
    c_bwq.wait()
    for c in c_bwo:
        c.wait()
    c_ax.wait()
    with jax.named_scope('ph1_v'):
        proj(wv2, vx, extra_v)
    c_awv.start()
    for c in (*c_awo, *c_bwot):
        c.start()
    c_ckv.wait(); c_awq.wait(); c_awk.wait()

    G = 4
    gr = lax.broadcasted_iota(jnp.int32, (G * MEM, G * (SEG + MEM)), 0) // MEM
    gc = lax.broadcasted_iota(jnp.int32, (G * MEM, G * (SEG + MEM)), 1)
    gvis = jnp.where(gc < G * SEG, gc // SEG, (gc - G * SEG) // MEM) == gr

    def mem_step(mem, s):
        q = _dot(mem, _w(wq2)) * QSCALE
        k = _dot(mem, _w(wk2))
        rows = pl.ds(pl.multiple_of(s * SEG, SEG), SEG)
        scs, vvs = [], []
        for g in range(H // G):
            cs = [slice(h * DH, (h + 1) * DH) for h in range(g * G, (g + 1) * G)]
            qg = jnp.concatenate([q[:, c] for c in cs], axis=0).astype(BF)
            km = jnp.concatenate([k[:, c] for c in cs], axis=0).astype(BF)
            kk = jnp.concatenate([kx[rows, c] for c in cs] + [km], axis=0)
            scs.append(jnp.where(gvis, _dot_nt(qg, kk), NEG))
        v = _dot(mem, _w(wv2))
        sc = jnp.concatenate(scs, axis=0)
        m = jnp.max(sc, axis=1, keepdims=True)
        p = jnp.exp2(sc - m)
        r = _recip(jnp.sum(p, axis=1, keepdims=True))
        p = p.astype(BF)
        ctx = []
        for g in range(H // G):
            cs = [slice(h * DH, (h + 1) * DH) for h in range(g * G, (g + 1) * G)]
            vm = jnp.concatenate([v[:, c] for c in cs], axis=0).astype(BF)
            vv = jnp.concatenate([vx[rows, c] for c in cs] + [vm], axis=0)
            gs = slice(g * G * MEM, (g + 1) * G * MEM)
            o = _dot(p[gs], vv) * r[gs]
            ctx += [o[j * MEM:(j + 1) * MEM] for j in range(G)]
        ctx = jnp.concatenate(ctx, axis=1).astype(BF)
        return _dot(ctx, _w(bwo)).astype(BF), k, v

    def rec_pair(p, mem):
        mem1, k0, v0 = mem_step(mem, 2 * p)
        mem2, k1, v1 = mem_step(mem1, 2 * p + 1)
        prow = pl.ds(pl.multiple_of(p * 16, 16), 16)
        kmem[prow, :] = jnp.concatenate([k0, k1], axis=0).astype(BF)
        vmem[prow, :] = jnp.concatenate([v0, v1], axis=0).astype(BF)
        return mem2

    with jax.named_scope('rec'):
        lax.fori_loop(0, NSEG // 2, rec_pair, mem0_ref[...])

    c_awv.wait()
    BQ = 128
    tri = (lax.broadcasted_iota(jnp.int32, (BQ, BQ), 1) <= lax.broadcasted_iota(jnp.int32, (BQ, BQ), 0))

    def head_pair(raw, rows, i):
        u = raw.bitcast(jnp.uint32)[0:rows, pl.ds(i, 1), :].reshape(rows, DH)
        lo = pltpu.bitcast(u << 16, F32).astype(BF)
        hi = pltpu.bitcast(u & jnp.uint32(0xFFFF0000), F32).astype(BF)
        return lo, hi

    def a_pair(i2, carry):
        wq = head_pair(raw0, DM, i2)
        wk = head_pair(raw1, DC, i2)
        wv = head_pair(raw2, DC, i2)
        NB = S // BQ

        q2 = (_dot(ax[...], jnp.concatenate(wq, axis=1)) * QSCALE).astype(BF)
        kv = _dot(ckv[...], jnp.concatenate([wk[0], wv[0], wk[1], wv[1]], axis=1)).astype(BF)

        def project(e):
            return q2[:, e * DH:(e + 1) * DH], kv[:, 2 * e * DH:(2 * e + 1) * DH], kv[:, (2 * e + 1) * DH:(2 * e + 2) * DH]

        def scores(qkv, i):
            q, k, _ = qkv
            r0 = i * BQ
            qi = q[r0:r0 + BQ]
            sc = jnp.where(tri, _dot_nt(qi, k[r0:r0 + BQ]), NEG)
            if i > 0:
                sc = jnp.concatenate([_dot_nt(qi, k[0:r0]), sc], axis=1)
            return sc

        def finish(qkv, e, i, sc):
            cols = pl.ds(pl.multiple_of(i2 * 2 * DH + e * DH, DH), DH)
            r0 = i * BQ
            m = jnp.max(sc, axis=1, keepdims=True)
            p = jnp.exp2(sc - m)
            l = jnp.sum(p, axis=1, keepdims=True)
            o = _dot(p.astype(BF), qkv[2][0:r0 + BQ])
            ctxa[r0:r0 + BQ, cols] = (o * _recip(l)).astype(BF)

        items = [(e, i) for e in range(2) for i in range(NB)]
        qkvs = {0: project(0)}
        sc = scores(qkvs[0], 0)
        for n, (e, i) in enumerate(items):
            nxt = None
            if n + 1 < len(items):
                e1, i1 = items[n + 1]
                if e1 not in qkvs:
                    qkvs[e1] = project(e1)
                nxt = scores(qkvs[e1], i1)
            finish(qkvs[e], e, i, sc)
            sc = nxt
        return carry
    with jax.named_scope('a_attn'):
        lax.fori_loop(0, H // 2, a_pair, 0)

    for c in (*c_awo, *c_bwot):
        c.wait()

    def a_out(r, carry):
        rows = pl.ds(pl.multiple_of(r * RB, RB), RB)
        o_ref[rows, 0:DM] = _dot_nt(awo[...], ctxa[rows, :]).T.astype(BF)
        return carry
    with jax.named_scope('a_out'):
        lax.fori_loop(0, S // RB, a_out, 0)

    T = 2
    ri = lax.broadcasted_iota(jnp.int32, (T * SEG, T * (SEG + MEM)), 0)
    ci = lax.broadcasted_iota(jnp.int32, (T * SEG, T * (SEG + MEM)), 1)
    xkey = ci < T * SEG
    cseg = jnp.where(xkey, ci // SEG, (ci - T * SEG) // MEM)
    vis = (cseg == ri // SEG) & (jnp.where(xkey, ci, 0) <= ri)

    NCH = 4
    TPC = NSEG // T // NCH

    def b_pair(i2, carry):
        pc = pl.ds(pl.multiple_of(i2 * 2 * DH, 2 * DH), 2 * DH)
        q2 = (_dot(bx[...], _w(wq2, cols=pc)) * QSCALE).astype(BF)

        def tiles(c):
            for t in range(c * TPC, (c + 1) * TPC):
                yield slice(t * T * SEG, (t + 1) * T * SEG), slice(t * T * MEM, (t + 1) * T * MEM)

        def scores(e, c):
            cols = pl.ds(pl.multiple_of(i2 * 2 * DH + e * DH, DH), DH)
            scs = []
            for xr, mr in tiles(c):
                kk = jnp.concatenate([kx[xr, cols], kmem[mr, cols]], axis=0)
                scs.append(jnp.where(vis, _dot_nt(q2[xr, e * DH:(e + 1) * DH], kk), NEG))
            return jnp.concatenate(scs, axis=0)

        def finish(e, c, sc):
            cols = pl.ds(pl.multiple_of(i2 * 2 * DH + e * DH, DH), DH)
            m = jnp.max(sc, axis=1, keepdims=True)
            p = jnp.exp2(sc - m)
            r = _recip(jnp.sum(p, axis=1, keepdims=True))
            p = p.astype(BF)
            for j, (xr, mr) in enumerate(tiles(c)):
                lr = slice(j * T * SEG, (j + 1) * T * SEG)
                vv = jnp.concatenate([vx[xr, cols], vmem[mr, cols]], axis=0)
                ctxa[xr, cols] = (_dot(p[lr], vv) * r[lr]).astype(BF)

        items = [(e, c) for e in range(2) for c in range(NCH)]
        sc = scores(*items[0])
        for n, it in enumerate(items):
            nxt = scores(*items[n + 1]) if n + 1 < len(items) else None
            finish(*it, sc)
            sc = nxt
        return carry
    with jax.named_scope('b_attn'):
        lax.fori_loop(0, H // 2, b_pair, 0)

    def b_out(r, carry):
        rows = pl.ds(pl.multiple_of(r * RB, RB), RB)
        o_ref[rows, DM:2 * DM] = _dot_nt(bwot[...], ctxa[rows, :]).T.astype(BF)
        pltpu.make_async_copy(o_ref.at[rows], o_hbm.at[rows], osems.at[r]).start()
        return carry
    with jax.named_scope('b_out'):
        lax.fori_loop(0, S // RB, b_out, 0)
    for r in range(S // RB):
        rows = pl.ds(r * RB, RB)
        pltpu.make_async_copy(o_ref.at[rows], o_hbm.at[rows], osems.at[r]).wait()


@jax.jit
def _run(A_x, A_c_kv, A_w_q, A_w_uk, A_w_uv, A_w_o, B_x, B_mem0, B_Wq, B_Wk, B_Wv, B_Wo):
    any_spec = pl.BlockSpec(memory_space=pl.ANY)
    vm = pltpu.VMEM
    out = pl.pallas_call(
        _kernel,
        out_shape=jax.ShapeDtypeStruct((S, 2 * DM), BF),
        in_specs=[any_spec] * 7 + [pl.BlockSpec(memory_space=pltpu.VMEM)] + [any_spec] * 4,
        out_specs=any_spec,
        scratch_shapes=[
            vm((S, DM), BF), vm((S, DC), BF), vm((S, DM), BF),
            vm((DM, H, DH), BF), vm((DM, H, DH), BF), vm((DM, H, DH), BF),
            vm((DM, HD), BF), vm((HD // 2, DM), jnp.uint32),
            vm((DM // 2, HD), jnp.uint32), vm((DM // 2, HD), jnp.uint32), vm((DM // 2, HD), jnp.uint32),
            vm((S, HD), BF), vm((S, HD), BF),
            vm((NSEG * MEM, HD), BF), vm((NSEG * MEM, HD), BF),
            vm((S, HD), BF),
            vm((S, 2 * DM), BF),
            vm((DM, HD), BF),
            pltpu.SemaphoreType.DMA((11,)),
            pltpu.SemaphoreType.DMA((2 * H,)),
            pltpu.SemaphoreType.DMA((4,)),
        ],
        compiler_params=pltpu.CompilerParams(vmem_limit_bytes=126 * 2 ** 20),
    )(A_x.reshape(S, DM).T, A_c_kv.reshape(S, DC), A_w_q, A_w_uk, A_w_uv, jnp.transpose(A_w_o, (0, 2, 1)),
      B_x.reshape(S, DM).T, B_mem0.reshape(MEM, DM), B_Wq, B_Wk, B_Wv, jnp.transpose(B_Wo, (0, 2, 1)))
    return out.reshape(1, S, 2 * DM)


def pallas_concat_heads__compressed_kv_cla__memory_aug_recurrent_mem_tr__prompt_kernel(
        A_x, A_c_kv, A_w_q, A_w_uk, A_w_uv, A_w_o, B_x, B_mem0, B_Wq, B_Wk, B_Wv, B_Wo, B_seg_len=SEG):
    del B_seg_len
    return _run(A_x, A_c_kv, A_w_q, A_w_uk, A_w_uv, A_w_o, B_x, B_mem0, B_Wq, B_Wk, B_Wv, B_Wo)
```
